```python
import jax
import jax.numpy as jnp

def _softmax(x, axis=-1):
    return jax.nn.softmax(x, axis=axis)
def _gelu(x):
    return jax.nn.gelu(x, approximate=True)
def _silu(x):
    return jax.nn.silu(x)
def _sigmoid(x):
    return jax.nn.sigmoid(x)
def _layernorm(x, axis=-1, eps=1e-5):
    m = jnp.mean(x, axis=axis, keepdims=True)
    v = jnp.var(x, axis=axis, keepdims=True)
    return (x - m) / jnp.sqrt(v + eps)
def _scatter_add(tgt, idx, src, axis=0):
    return tgt.at[idx].add(src)
def _segment_sum(src, seg, n):
    return jax.ops.segment_sum(src, seg, n)
class _Rng:
    def __init__(self, key):
        self._k = key
    def _next(self):
        self._k, sub = jax.random.split(self._k)
        return sub
    def normal(self, shape):
        return jax.random.normal(self._next(), shape, dtype=jnp.bfloat16)
    def randint(self, lo, hi, shape):
        return jax.random.randint(self._next(), shape, lo, hi, dtype=jnp.int32)
    def uniform(self, shape, lo=0.0, hi=1.0):
        return jax.random.uniform(self._next(), shape, jnp.bfloat16, lo, hi)
    def permutation(self, n):
        return jax.random.permutation(self._next(), n)


kernel_name = 'gated_mix__sliding_block_cached__moe_arch_mod__decode'

def setup_inputs():
    _rng = _Rng(jax.random.key(int.from_bytes(__import__("os").urandom(4), "little")))
    _w = (lambda a: (lambda t: t.astype(jnp.bfloat16) if jnp.issubdtype(t.dtype, jnp.floating) else t)(jnp.asarray(a)))
    def _A_setup():
        B, Sq, D = 1, 1, 640
        Hq, Hkv, Sk, Dh = 32, 32, 32768, 192
        assert Hq % Hkv == 0, (Hq, Hkv)
        return {
            "x": _w((lambda *s: _rng.normal(s) * 0.05)(B, Sq, D)),
            "k_cache": _w((lambda *s: _rng.normal(s) * 0.05)(B, Hkv, Sk, Dh)),
            "v_cache": _w((lambda *s: _rng.normal(s) * 0.05)(B, Hkv, Sk, Dh)),
            "wq": _w((lambda *s: _rng.normal(s) * 0.05)(D, Hq * Dh) * (D ** -0.5)),
            "wo": _w((lambda *s: _rng.normal(s) * 0.05)(Hq * Dh, D) * ((Hq * Dh) ** -0.5)),
        }
    _A_in = _A_setup()

    def _B_setup():
        B, S, D, F, C = 1, 1, 640, 1536, 1
        return {
            "x": _w((lambda *s: _rng.normal(s) * 0.05)(B, S, D)),
            "w_r": _w((lambda *s: _rng.normal(s) * 0.05)(D)),
            "w_gate": _w((lambda *s: _rng.normal(s) * 0.05)(D, F)),
            "w_up": _w((lambda *s: _rng.normal(s) * 0.05)(D, F)),
            "w_down": _w((lambda *s: _rng.normal(s) * 0.05)(F, D)),
        }
    _B_in = _B_setup()

    return {
        "A_x": _A_in["x"],
        "A_k_cache": _A_in["k_cache"],
        "A_v_cache": _A_in["v_cache"],
        "A_wq": _A_in["wq"],
        "A_wo": _A_in["wo"],
        "B_x": _B_in["x"],
        "B_w_r": _B_in["w_r"],
        "B_w_gate": _B_in["w_gate"],
        "B_w_up": _B_in["w_up"],
        "B_w_down": _B_in["w_down"],
        "gate_w": _w((lambda *s: _rng.normal(s) * 0.05)(640)),
    }

def reference(A_x, A_k_cache, A_v_cache, A_wq, A_wo, B_x, B_w_r, B_w_gate, B_w_up, B_w_down, gate_w):
    def _A_ref(x, k_cache, v_cache, wq, wo):
        B, Sq, D = x.shape
        Hq, Dh = 32, 192
        Hkv, Sk = k_cache.shape[1], k_cache.shape[2]
        W = min(4096, max(256, Sk // 4))
        rep = Hq // Hkv
        q = (lambda x, *d: x.transpose(*d))((x @ wq).reshape(B, Sq, Hq, Dh), 0, 2, 1, 3)
        k = jnp.repeat(k_cache[:, :, Sk - W:, :], rep, axis=1)
        v = jnp.repeat(v_cache[:, :, Sk - W:, :], rep, axis=1)
        scores = jnp.einsum("bhqd,bhkd->bhqk", q, k) * (Dh ** -0.5)
        p = _softmax(scores, axis=-1)
        o = jnp.einsum("bhqk,bhkd->bhqd", p, v)
        return (lambda x, *d: x.transpose(*d))(o, 0, 2, 1, 3).reshape(B, Sq, Hq * Dh) @ wo

    def _B_ref(x, w_r, w_gate, w_up, w_down):
        B, S, D = x.shape
        C = 1
        r = x @ w_r
        idx = jnp.argsort(-r, axis=-1)[:, :C]
        idx_e = jnp.repeat(idx.reshape(B, C, 1), D, axis=2)
        x_sel = jnp.take_along_axis(x, idx_e, axis=1)
        g = _silu(x_sel @ w_gate)
        u = x_sel @ w_up
        y = (g * u) @ w_down
        r_sel = _sigmoid(jnp.take_along_axis(r, idx, axis=1))
        y = y * r_sel.reshape(B, C, 1)
        b_off = (jnp.arange(B) * S).reshape(B, 1)
        flat_idx = (idx + b_off).reshape(B * C)
        zero = (x * 0.0).reshape(B * S, D)
        upd = _scatter_add(zero, flat_idx, y.reshape(B * C, D), axis=0)
        return x + upd.reshape(B, S, D)

    x = A_x
    g = _sigmoid((x * gate_w).sum(-1, keepdims=True))
    a = _A_ref(x, A_k_cache, A_v_cache, A_wq, A_wo)
    b = _B_ref(x, B_w_r, B_w_gate, B_w_up, B_w_down)
    return g * a + (1 - g) * b
```

```python
import functools
import jax
import jax.numpy as jnp
import numpy as np
from jax import lax
import jax.experimental.pallas as pl
import jax.experimental.pallas.tpu as pltpu

H, DH, D, F = 32, 192, 640, 1536
f32, bf16 = jnp.float32, jnp.bfloat16


def build(HPC=2, NB=4, vmem_mb=100):
    R = HPC * DH
    NCH = H // HPC

    def kernel(x_hbm, kT_hbm, vT_hbm, wq_hbm, wo_hbm, wr_hbm, wg_hbm, wu_hbm, wd_hbm, gw_hbm,
               out_ref,
               x_v, wr_v, gw_v, wq_v, wo_v, wg_v, wu_v, wd_v, kbuf, vbuf, q_scr,
               sem_small, sem_w, sem_k, sem_v):
        SK = kT_hbm.shape[1]
        W = min(4096, max(256, SK // 4))
        S0 = SK - W

        def k_copy(j, slot):
            return pltpu.make_async_copy(
                kT_hbm.at[pl.ds(j * R, R), pl.ds(S0, W)], kbuf.at[slot], sem_k.at[slot])

        def v_copy(j, slot):
            return pltpu.make_async_copy(
                vT_hbm.at[pl.ds(j * R, R), pl.ds(S0, W)], vbuf.at[slot], sem_v.at[slot])

        c_x = pltpu.make_async_copy(x_hbm, x_v, sem_small.at[0])
        c_wr = pltpu.make_async_copy(wr_hbm, wr_v, sem_small.at[1])
        c_gw = pltpu.make_async_copy(gw_hbm, gw_v, sem_small.at[2])
        c_wq = pltpu.make_async_copy(wq_hbm, wq_v, sem_w.at[0])
        c_wo = pltpu.make_async_copy(wo_hbm, wo_v, sem_w.at[1])
        c_wg = pltpu.make_async_copy(wg_hbm, wg_v, sem_w.at[2])
        c_wu = pltpu.make_async_copy(wu_hbm, wu_v, sem_w.at[3])
        c_wd = pltpu.make_async_copy(wd_hbm, wd_v, sem_w.at[4])
        c_x.start(); c_wr.start(); c_gw.start()
        c_wq.start()
        for j in range(NB - 1):
            k_copy(j, j).start()
            v_copy(j, j).start()
        c_wo.start()
        c_wg.start(); c_wu.start(); c_wd.start()

        c_x.wait(); c_wr.wait(); c_gw.wait()
        xf = x_v[0].astype(f32)
        x8 = jnp.broadcast_to(xf, (8, D)).astype(bf16)
        wr = wr_v[...].astype(f32).reshape(1, D)
        gw = gw_v[...].astype(f32).reshape(1, D)
        r = jnp.sum(xf * wr, axis=1, keepdims=True)
        gate = jax.nn.sigmoid(jnp.sum(xf * gw, axis=1, keepdims=True))
        r_sel = jax.nn.sigmoid(r)

        c_wq.wait()
        row = lax.broadcasted_iota(jnp.int32, (8, R), 0)
        col = lax.broadcasted_iota(jnp.int32, (8, R), 1)
        mask = (col >= row * DH) & (col < (row + 1) * DH)
        for j in range(NCH):
            qj = jnp.dot(x8, wq_v[:, j * R:(j + 1) * R], preferred_element_type=f32)
            q_scr[j] = jnp.where(mask, qj, 0.0).astype(bf16)

        c_wo.wait()
        scale = np.float32(DH ** -0.5)

        def body(j, acc):
            slot = j % NB
            nj = j + NB - 1

            @pl.when(nj < NCH)
            def _():
                ns = nj % NB
                k_copy(nj, ns).start()
                v_copy(nj, ns).start()

            k_copy(j, slot).wait()
            s = jnp.dot(q_scr[j], kbuf[slot], preferred_element_type=f32) * scale
            m = jnp.max(s, axis=1, keepdims=True)
            p = jnp.exp(s - m)
            l = jnp.sum(p, axis=1, keepdims=True)
            v_copy(j, slot).wait()
            o = lax.dot_general(p.astype(bf16), vbuf[slot], (((1,), (1,)), ((), ())),
                                preferred_element_type=f32)
            o = jnp.where(mask, o / l, 0.0).astype(bf16)
            return acc + jnp.dot(o, wo_v[j], preferred_element_type=f32)

        acc = lax.fori_loop(0, NCH, body, jnp.zeros((8, D), f32))
        a = jnp.sum(acc, axis=0, keepdims=True)

        c_wg.wait(); c_wu.wait()
        g = jnp.dot(x8, wg_v[...], preferred_element_type=f32)
        u = jnp.dot(x8, wu_v[...], preferred_element_type=f32)
        h = (jax.nn.silu(g) * u).astype(bf16)
        c_wd.wait()
        y = jnp.dot(h, wd_v[...], preferred_element_type=f32)[0:1]
        b = xf + (xf * 0.0 + y * r_sel)
        res = gate * a + (1.0 - gate) * b
        out_ref[0] = res.astype(bf16)

    def fn(A_x, A_k_cache, A_v_cache, A_wq, A_wo, B_x, B_w_r, B_w_gate, B_w_up, B_w_down, gate_w):
        SK = A_k_cache.shape[2]
        W = min(4096, max(256, SK // 4))
        kT = A_k_cache.transpose(0, 1, 3, 2).reshape(H * DH, SK)
        vT = A_v_cache.transpose(0, 1, 3, 2).reshape(H * DH, SK)
        wo = A_wo.reshape(NCH, R, D)
        hbm = pl.BlockSpec(memory_space=pl.ANY)
        return pl.pallas_call(
            kernel,
            out_shape=jax.ShapeDtypeStruct((1, 1, D), bf16),
            in_specs=[hbm] * 10,
            out_specs=pl.BlockSpec(memory_space=pltpu.VMEM),
            scratch_shapes=[
                pltpu.VMEM((1, 1, D), bf16),
                pltpu.VMEM((D,), bf16),
                pltpu.VMEM((D,), bf16),
                pltpu.VMEM((D, H * DH), bf16),
                pltpu.VMEM((NCH, R, D), bf16),
                pltpu.VMEM((D, F), bf16),
                pltpu.VMEM((D, F), bf16),
                pltpu.VMEM((F, D), bf16),
                pltpu.VMEM((NB, R, W), bf16),
                pltpu.VMEM((NB, R, W), bf16),
                pltpu.VMEM((NCH, 8, R), bf16),
                pltpu.SemaphoreType.DMA((3,)),
                pltpu.SemaphoreType.DMA((5,)),
                pltpu.SemaphoreType.DMA((NB,)),
                pltpu.SemaphoreType.DMA((NB,)),
            ],
            compiler_params=pltpu.CompilerParams(vmem_limit_bytes=vmem_mb * 1024 * 1024),
        )(A_x, kT, vT, A_wq, wo, B_w_r, B_w_gate, B_w_up, B_w_down, gate_w)
    return jax.jit(fn)


_impl = build(2, 3)


@jax.jit
def pallas_gated_mix__sliding_block_cached__moe_arch_mod__decode_kernel(
    A_x, A_k_cache, A_v_cache, A_wq, A_wo, B_x, B_w_r, B_w_gate, B_w_up, B_w_down, gate_w,
):
    return _impl(A_x, A_k_cache, A_v_cache, A_wq, A_wo, B_x, B_w_r, B_w_gate, B_w_up, B_w_down, gate_w)
```

```python
import jax
import jax.numpy as jnp
import numpy as np
from jax import lax
import jax.experimental.pallas as pl
import jax.experimental.pallas.tpu as pltpu

H, DH = 32, 192
HPC = 2
R = HPC * DH
NCH = H // HPC
NB = 3
NWD = 4
F32, BF16 = jnp.float32, jnp.bfloat16


def _window(sk):
    return min(4096, max(256, sk // 4))


def _kernel(x_hbm, kT_hbm, vT_hbm, wq_hbm, wo_hbm, wr_hbm, wg_hbm, wu_hbm, wd_hbm, gw_hbm,
            out_ref,
            x_v, wr_v, gw_v, wq_v, wo_v, wg_v, wu_v, wd_v, k_v, v_v, q_scr, h_scr,
            sem_w, sem_r):
    D = x_hbm.shape[-1]
    SK = kT_hbm.shape[1]
    W = _window(SK)
    S0 = SK - W
    RD = wd_hbm.shape[1]

    def chunk_copies(j, slot):
        rows = pl.ds(j * R, R)
        cols = pl.ds(S0, W)
        return (
            pltpu.make_async_copy(kT_hbm.at[rows, cols], k_v.at[slot], sem_r.at[slot]),
            pltpu.make_async_copy(vT_hbm.at[rows, cols], v_v.at[slot], sem_r.at[slot]),
            pltpu.make_async_copy(wo_hbm.at[j], wo_v.at[slot], sem_r.at[slot]),
        )

    def start_chunk(j, slot):
        for c in chunk_copies(j, slot):
            c.start()

    def wait_chunk(j, slot):
        for c in chunk_copies(j, slot):
            c.wait()

    def down_copy(c):
        return pltpu.make_async_copy(wd_hbm.at[c], wd_v.at[c], sem_r.at[c])

    head_copies = (
        pltpu.make_async_copy(wq_hbm, wq_v, sem_w),
        pltpu.make_async_copy(x_hbm, x_v, sem_w),
        pltpu.make_async_copy(wr_hbm, wr_v, sem_w),
        pltpu.make_async_copy(gw_hbm, gw_v, sem_w),
    )
    ffn_copies = (
        pltpu.make_async_copy(wg_hbm, wg_v, sem_w),
        pltpu.make_async_copy(wu_hbm, wu_v, sem_w),
    )

    for c in head_copies:
        c.start()

    def prime(j, carry):
        start_chunk(j, j)
        return carry

    lax.fori_loop(0, NB, prime, 0)

    for c in head_copies:
        c.wait()

    xf = x_v[0].astype(F32)
    x8 = jnp.broadcast_to(xf, (8, D)).astype(BF16)
    gate = jax.nn.sigmoid(
        jnp.sum(xf * gw_v[...].astype(F32).reshape(1, D), axis=1, keepdims=True))
    r_sel = jax.nn.sigmoid(
        jnp.sum(xf * wr_v[...].astype(F32).reshape(1, D), axis=1, keepdims=True))

    row = lax.broadcasted_iota(jnp.int32, (8, R), 0)
    col = lax.broadcasted_iota(jnp.int32, (8, R), 1)
    own = (col >= row * DH) & (col < (row + 1) * DH)

    def q_body(j, carry):
        off = pl.multiple_of(j * R, 128)
        qj = jnp.dot(x8, wq_v[:, pl.ds(off, R)], preferred_element_type=F32)
        q_scr[j] = jnp.where(own, qj, 0.0).astype(BF16)
        return carry

    lax.fori_loop(0, NCH, q_body, 0)

    scale = np.float32(DH ** -0.5)

    def body(j, acc):
        slot = j % NB
        wait_chunk(j, slot)
        s = jnp.dot(q_scr[j], k_v[slot], preferred_element_type=F32) * scale
        m = jnp.max(s, axis=1, keepdims=True)
        p = jnp.exp(s - m)
        l = jnp.sum(p, axis=1, keepdims=True)
        o = lax.dot_general(p.astype(BF16), v_v[slot], (((1,), (1,)), ((), ())),
                            preferred_element_type=F32)
        o = jnp.where(own, o / l, 0.0).astype(BF16)
        acc = acc + jnp.dot(o, wo_v[slot], preferred_element_type=F32)

        @pl.when(j + NB < NCH)
        def _():
            start_chunk(j + NB, slot)

        @pl.when(j + NB == NCH)
        def _():
            for c in ffn_copies:
                c.start()

        return acc

    acc = lax.fori_loop(0, NCH, body, jnp.zeros((8, D), F32))

    def start_down(c, carry):
        down_copy(c).start()
        return carry

    lax.fori_loop(0, NWD, start_down, 0)

    a = jnp.sum(acc, axis=0, keepdims=True)
    c0 = gate * a + (1.0 - gate) * (xf + xf * 0.0)
    c1 = (1.0 - gate) * r_sel

    for c in ffn_copies:
        c.wait()

    def h_body(c, carry):
        off = pl.multiple_of(c * RD, 128)
        g = jnp.dot(x8, wg_v[:, pl.ds(off, RD)], preferred_element_type=F32)
        u = jnp.dot(x8, wu_v[:, pl.ds(off, RD)], preferred_element_type=F32)
        h_scr[c] = (jax.nn.silu(g) * u).astype(BF16)
        return carry

    lax.fori_loop(0, NWD, h_body, 0)

    def y_body(c, y):
        down_copy(c).wait()
        return y + jnp.dot(h_scr[c], wd_v[c], preferred_element_type=F32)

    y = lax.fori_loop(0, NWD, y_body, jnp.zeros((8, D), F32))

    out_ref[0] = (c0 + c1 * y[0:1]).astype(BF16)


@jax.jit
def pallas_gated_mix__sliding_block_cached__moe_arch_mod__decode_kernel(
    A_x: jax.Array,
    A_k_cache: jax.Array,
    A_v_cache: jax.Array,
    A_wq: jax.Array,
    A_wo: jax.Array,
    B_x: jax.Array,
    B_w_r: jax.Array,
    B_w_gate: jax.Array,
    B_w_up: jax.Array,
    B_w_down: jax.Array,
    gate_w: jax.Array,
):
    del B_x
    D = A_x.shape[-1]
    F = B_w_gate.shape[1]
    SK = A_k_cache.shape[2]
    W = _window(SK)
    RD = F // NWD
    assert A_x.shape == (1, 1, D) and A_k_cache.shape == (1, H, SK, DH)
    assert F % (NWD * 128) == 0

    kT = A_k_cache.transpose(0, 1, 3, 2).reshape(H * DH, SK)
    vT = A_v_cache.transpose(0, 1, 3, 2).reshape(H * DH, SK)
    wo = A_wo.reshape(NCH, R, D)
    wd = B_w_down.reshape(NWD, RD, D)

    hbm = pl.BlockSpec(memory_space=pl.ANY)
    return pl.pallas_call(
        _kernel,
        out_shape=jax.ShapeDtypeStruct((1, 1, D), BF16),
        in_specs=[hbm] * 10,
        out_specs=pl.BlockSpec(memory_space=pltpu.VMEM),
        scratch_shapes=[
            pltpu.VMEM((1, 1, D), BF16),
            pltpu.VMEM((D,), BF16),
            pltpu.VMEM((D,), BF16),
            pltpu.VMEM((D, H * DH), BF16),
            pltpu.VMEM((NB, R, D), BF16),
            pltpu.VMEM((D, F), BF16),
            pltpu.VMEM((D, F), BF16),
            pltpu.VMEM((NWD, RD, D), BF16),
            pltpu.VMEM((NB, R, W), BF16),
            pltpu.VMEM((NB, R, W), BF16),
            pltpu.VMEM((NCH, 8, R), BF16),
            pltpu.VMEM((NWD, 8, RD), BF16),
            pltpu.SemaphoreType.DMA(()),
            pltpu.SemaphoreType.DMA((max(NB, NWD),)),
        ],
        compiler_params=pltpu.CompilerParams(vmem_limit_bytes=56 * 1024 * 1024),
    )(A_x, kT, vT, A_wq, wo, B_w_r, B_w_gate, B_w_up, wd, gate_w)
```

```python
import jax
import jax.numpy as jnp
import numpy as np
from jax import lax
import jax.experimental.pallas as pl
import jax.experimental.pallas.tpu as pltpu

H, DH = 32, 192
HPC = 2
R = HPC * DH
NCH = H // HPC
NB = 3
NF = 4
WD_GROUPS = ((1, 1024), (2, 256))
F32, BF16 = jnp.float32, jnp.bfloat16


def _window(sk):
    return min(4096, max(256, sk // 4))


def _kernel(x_hbm, kT_hbm, vT_hbm, wq_hbm, wo_hbm, wr_hbm, wg_hbm, wu_hbm, wd_hbm, gw_hbm,
            out_ref,
            x_v, wr_v, gw_v, wq_v, wo_v, wg_v, wu_v, wd_v, k_v, v_v, q_scr, h_scr,
            sem_w, sem_r):
    D = x_hbm.shape[-1]
    SK = kT_hbm.shape[1]
    W = _window(SK)
    S0 = SK - W
    F = wd_hbm.shape[0]
    RF = F // NF

    def chunk_copies(j, slot):
        rows = pl.ds(j * R, R)
        cols = pl.ds(S0, W)
        return (
            pltpu.make_async_copy(kT_hbm.at[rows, cols], k_v.at[slot], sem_r.at[slot]),
            pltpu.make_async_copy(vT_hbm.at[rows, cols], v_v.at[slot], sem_r.at[slot]),
            pltpu.make_async_copy(wo_hbm.at[j], wo_v.at[slot], sem_r.at[slot]),
        )

    def start_chunk(j, slot):
        for c in chunk_copies(j, slot):
            c.start()

    def wait_chunk(j, slot):
        for c in chunk_copies(j, slot):
            c.wait()

    def down_copy(row0, sem0, c, rows):
        sl = pl.ds(pl.multiple_of(row0 + c * rows, 128), rows)
        return pltpu.make_async_copy(wd_hbm.at[sl], wd_v.at[sl], sem_r.at[sem0 + c])

    head_copies = (
        pltpu.make_async_copy(wq_hbm, wq_v, sem_w),
        pltpu.make_async_copy(x_hbm, x_v, sem_w),
        pltpu.make_async_copy(wr_hbm, wr_v, sem_w),
        pltpu.make_async_copy(gw_hbm, gw_v, sem_w),
    )
    ffn_copies = (
        pltpu.make_async_copy(wg_hbm, wg_v, sem_w),
        pltpu.make_async_copy(wu_hbm, wu_v, sem_w),
    )

    for c in head_copies:
        c.start()

    def prime(j, carry):
        start_chunk(j, j)
        return carry

    lax.fori_loop(0, NB, prime, 0)

    for c in head_copies:
        c.wait()

    xf = x_v[0].astype(F32)
    x8 = jnp.broadcast_to(xf, (8, D)).astype(BF16)
    gate = jax.nn.sigmoid(
        jnp.sum(xf * gw_v[...].astype(F32).reshape(1, D), axis=1, keepdims=True))
    r_sel = jax.nn.sigmoid(
        jnp.sum(xf * wr_v[...].astype(F32).reshape(1, D), axis=1, keepdims=True))

    row = lax.broadcasted_iota(jnp.int32, (8, R), 0)
    col = lax.broadcasted_iota(jnp.int32, (8, R), 1)
    own = (col >= row * DH) & (col < (row + 1) * DH)

    def q_body(j, carry):
        off = pl.multiple_of(j * R, 128)
        qj = jnp.dot(x8, wq_v[:, pl.ds(off, R)], preferred_element_type=F32)
        q_scr[j] = jnp.where(own, qj, 0.0).astype(BF16)
        return carry

    lax.fori_loop(0, NCH, q_body, 0)

    scale = np.float32(DH ** -0.5)

    def body(j, acc):
        slot = j % NB
        wait_chunk(j, slot)
        s = jnp.dot(q_scr[j], k_v[slot], preferred_element_type=F32) * scale
        m = jnp.max(s, axis=1, keepdims=True)
        p = jnp.exp(s - m)
        l = jnp.sum(p, axis=1, keepdims=True)
        o = lax.dot_general(p.astype(BF16), v_v[slot], (((1,), (1,)), ((), ())),
                            preferred_element_type=F32)
        o = jnp.where(own, o / l, 0.0).astype(BF16)
        acc = acc + jnp.dot(o, wo_v[slot], preferred_element_type=F32)

        @pl.when(j + NB < NCH)
        def _():
            start_chunk(j + NB, slot)

        @pl.when(j + NB == NCH)
        def _():
            for c in ffn_copies:
                c.start()

        return acc

    acc = lax.fori_loop(0, NCH, body, jnp.zeros((8, D), F32))

    row0 = sem0 = 0
    for n, rows in WD_GROUPS:
        def start_down(c, carry, row0=row0, sem0=sem0, rows=rows):
            down_copy(row0, sem0, c, rows).start()
            return carry

        lax.fori_loop(0, n, start_down, 0)
        row0 += n * rows
        sem0 += n

    a = jnp.sum(acc, axis=0, keepdims=True)
    c0 = gate * a + (1.0 - gate) * (xf + xf * 0.0)
    c1 = (1.0 - gate) * r_sel

    for c in ffn_copies:
        c.wait()

    def h_body(c, carry):
        sl = pl.ds(pl.multiple_of(c * RF, 128), RF)
        g = jnp.dot(x8, wg_v[:, sl], preferred_element_type=F32)
        u = jnp.dot(x8, wu_v[:, sl], preferred_element_type=F32)
        h_scr[:, sl] = (jax.nn.silu(g) * u).astype(BF16)
        return carry

    lax.fori_loop(0, NF, h_body, 0)

    y = jnp.zeros((8, D), F32)
    row0 = sem0 = 0
    for n, rows in WD_GROUPS:
        def y_body(c, y, row0=row0, sem0=sem0, rows=rows):
            down_copy(row0, sem0, c, rows).wait()
            sl = pl.ds(pl.multiple_of(row0 + c * rows, 128), rows)
            return y + jnp.dot(h_scr[:, sl], wd_v[sl, :], preferred_element_type=F32)

        y = lax.fori_loop(0, n, y_body, y)
        row0 += n * rows
        sem0 += n

    out_ref[0] = (c0 + c1 * y[0:1]).astype(BF16)


@jax.jit
def pallas_gated_mix__sliding_block_cached__moe_arch_mod__decode_kernel(
    A_x: jax.Array,
    A_k_cache: jax.Array,
    A_v_cache: jax.Array,
    A_wq: jax.Array,
    A_wo: jax.Array,
    B_x: jax.Array,
    B_w_r: jax.Array,
    B_w_gate: jax.Array,
    B_w_up: jax.Array,
    B_w_down: jax.Array,
    gate_w: jax.Array,
):
    del B_x
    D = A_x.shape[-1]
    F = B_w_gate.shape[1]
    SK = A_k_cache.shape[2]
    W = _window(SK)
    assert A_x.shape == (1, 1, D) and A_k_cache.shape == (1, H, SK, DH)
    assert F % (NF * 128) == 0 and sum(n * r for n, r in WD_GROUPS) == F

    kT = A_k_cache.transpose(0, 1, 3, 2).reshape(H * DH, SK)
    vT = A_v_cache.transpose(0, 1, 3, 2).reshape(H * DH, SK)
    wo = A_wo.reshape(NCH, R, D)

    hbm = pl.BlockSpec(memory_space=pl.ANY)
    return pl.pallas_call(
        _kernel,
        out_shape=jax.ShapeDtypeStruct((1, 1, D), BF16),
        in_specs=[hbm] * 10,
        out_specs=pl.BlockSpec(memory_space=pltpu.VMEM),
        scratch_shapes=[
            pltpu.VMEM((1, 1, D), BF16),
            pltpu.VMEM((D,), BF16),
            pltpu.VMEM((D,), BF16),
            pltpu.VMEM((D, H * DH), BF16),
            pltpu.VMEM((NB, R, D), BF16),
            pltpu.VMEM((D, F), BF16),
            pltpu.VMEM((D, F), BF16),
            pltpu.VMEM((F, D), BF16),
            pltpu.VMEM((NB, R, W), BF16),
            pltpu.VMEM((NB, R, W), BF16),
            pltpu.VMEM((NCH, 8, R), BF16),
            pltpu.VMEM((8, F), BF16),
            pltpu.SemaphoreType.DMA(()),
            pltpu.SemaphoreType.DMA((max(NB, sum(n for n, _ in WD_GROUPS)),)),
        ],
        compiler_params=pltpu.CompilerParams(vmem_limit_bytes=56 * 1024 * 1024),
    )(A_x, kT, vT, A_wq, wo, B_w_r, B_w_gate, B_w_up, B_w_down, gate_w)
```
